```python
import os as _os
_os.environ.setdefault("JAX_PLATFORMS", "cpu")
import jax
import jax.numpy as jnp

def _softmax(x, axis=-1):
    return jax.nn.softmax(x, axis=axis)
def _gelu(x):
    return jax.nn.gelu(x, approximate=True)
def _silu(x):
    return jax.nn.silu(x)
def _sigmoid(x):
    return jax.nn.sigmoid(x)
def _layernorm(x, axis=-1, eps=1e-5):
    m = jnp.mean(x, axis=axis, keepdims=True)
    v = jnp.var(x, axis=axis, keepdims=True)
    return (x - m) / jnp.sqrt(v + eps)
def _scatter_add(tgt, idx, src, axis=0):
    return tgt.at[idx].add(src)
def _segment_sum(src, seg, n):
    return jax.ops.segment_sum(src, seg, n)
class _Rng:
    def __init__(self, key):
        self._k = key
    def _next(self):
        self._k, sub = jax.random.split(self._k)
        return sub
    def normal(self, shape):
        return jax.random.normal(self._next(), shape, dtype=jnp.bfloat16)
    def randint(self, lo, hi, shape):
        return jax.random.randint(self._next(), shape, lo, hi, dtype=jnp.int32)
    def uniform(self, shape, lo=0.0, hi=1.0):
        return jax.random.uniform(self._next(), shape, jnp.bfloat16, lo, hi)
    def permutation(self, n):
        return jax.random.permutation(self._next(), n)


kernel_name = 'standalone__cross_network_dcn_v2__recsys'

def setup_inputs():
    _rng = _Rng(jax.random.key(int.from_bytes(__import__("os").urandom(4), "little")))
    _w = (lambda a: (lambda t: t.astype(jnp.bfloat16) if jnp.issubdtype(t.dtype, jnp.floating) else t)(jnp.asarray(a)))
    B, F, D, L = 16384, 26, 16, 6
    Din = min(F * D, 512)
    R = max(Din // 4, 2)
    sc = Din ** -0.5
    return {
        "x0": _w((lambda *s: _rng.normal(s) * 0.05)(B, Din)),
        "U":  _w((lambda *s: _rng.normal(s) * 1.6)(L, Din, R) * sc),
        "V":  _w((lambda *s: _rng.normal(s) * 1.6)(L, R, Din) * sc),
        "bs": _w((lambda *s: _rng.normal(s) * 0.05)(L, Din)),
    }

def reference(x0, U, V, bs):
    x = x0
    for l in range(U.shape[0]):
        h = jnp.einsum('rd,bd->br', V[l], x)
        h = jnp.einsum('dr,br->bd', U[l], h)
        x = x0 * (h + bs[l]) + x
    return x
```

```python
import jax
import jax.numpy as jnp
from jax import lax
import jax.experimental.pallas as pl
import jax.experimental.pallas.tpu as pltpu

F32 = jnp.float32
BF16 = jnp.bfloat16

MXU = 128
SET = 512
PIECE = 16
FIRST = 2
PER = 6


def _dot(a, b):
    return lax.dot_general(a, b, (((1,), (0,)), ((), ())), preferred_element_type=F32)


def _schedule(nsets, nlayers):
    phases = [[], []]
    for s in range(nsets):
        for l in range(nlayers):
            phases[s % 2] += [("V", s, l), ("U", s, l)]
    order = []
    for t in range(max(len(phases[0]), len(phases[1]) + 1)):
        a = phases[0][t] if t < len(phases[0]) else None
        b = phases[1][t - 1] if 0 <= t - 1 < len(phases[1]) else None
        v = [("V", p[1], p[2], 0) for p in (a, b) if p and p[0] == "V"]
        u = [p for p in (a, b) if p and p[0] == "U"]
        u0 = [("U", p[1], p[2], 0) for p in u]
        u1 = [("U", p[1], p[2], 1) for p in u]
        order += (v + u0 + u1) if t == 1 else (u0 + v + u1)
    return order


def _kernel(x_hbm, u_hbm, v_hbm, b_hbm, o_hbm,
            xbuf, obuf, u_ref, v_ref, b_ref, vm_ref, l2_ref, vb_ref, xsem, osem, wsem):
    L, D, R = u_hbm.shape
    NS = xbuf.shape[0]
    KM = (D // MXU) * MXU
    rem = D - KM
    NF = MXU - R - 1
    NP = D - KM - NF
    G = SET // MXU
    half = D // 2

    def cols(i):
        return pl.ds(i * SET, SET) if isinstance(i, int) else pl.ds(pl.multiple_of(i * SET, SET), SET)

    def x_copy(i, s):
        return pltpu.make_async_copy(x_hbm.at[:, cols(i)], xbuf.at[i], xsem.at[s])

    def o_copy(i):
        return pltpu.make_async_copy(obuf.at[i], o_hbm.at[:, cols(i)], osem.at[0])

    def w_copies(j):
        sl = pl.ds(0, 1) if j == 0 else pl.ds(1, L - 1)
        copies = [pltpu.make_async_copy(v_hbm.at[sl], v_ref.at[sl], wsem.at[j]),
                  pltpu.make_async_copy(u_hbm.at[sl], u_ref.at[sl], wsem.at[j])]
        if j == 0:
            copies.append(pltpu.make_async_copy(b_hbm, b_ref, wsem.at[j]))
        return copies

    def prepare(l, b_t):
        v = v_ref[l].astype(F32)
        vm_ref[l] = v[:, :KM]
        vrem = jnp.concatenate([v[:, KM:], jnp.zeros((R, MXU - rem), F32)], axis=1)
        for p in range(NP):
            vb_ref[l, p] = jnp.broadcast_to(vrem[:, NF + p:NF + p + 1], (R, MXU))
        lane = lax.broadcasted_iota(jnp.int32, (R, MXU), 1)
        row = lax.broadcasted_iota(jnp.int32, (R, MXU), 0)
        eye = (lane == row + (NF + 1)).astype(F32)
        rhs = jnp.where(lane < NF, vrem, eye).astype(BF16)
        u = u_ref[l].astype(F32)
        q = D // 4
        w = jnp.concatenate([_dot(u[j * q:(j + 1) * q], rhs) for j in range(4)], axis=0)
        lane_d = lax.broadcasted_iota(jnp.int32, (D, MXU), 1)
        w = jnp.where(lane_d == NF, b_t[:, l:l + 1], w).astype(BF16)
        l2_ref[l, :rem] = w[KM:]
        l2_ref[l, rem:] = w[:KM]

    rows = list(range(KM, D, PIECE)) + list(range(0, KM, PIECE))
    nrem = rem // PIECE

    def block(base, nsets, first):
        x0, x, rhs2 = {}, {}, {}
        prepared = set()
        b_t = jnp.transpose(b_ref[...].astype(F32)) if first else None
        for op, s, l, c in _schedule(nsets, L):
            i = base + s
            if op == "V":
                if first and l not in prepared:
                    if l == 1:
                        for cp in w_copies(1):
                            cp.wait()
                    prepare(l, b_t)
                    prepared.add(l)
                if l == 0:
                    raw = [xbuf[i, r:r + PIECE, :] for r in rows]
                    x0[s] = [a.astype(F32) for a in raw]
                    x[s] = x0[s][:nrem] + raw[nrem:]
                xr = jnp.concatenate(x[s][:nrem], axis=0)
                acc = None
                for p in range(NP):
                    t = jnp.concatenate([vb_ref[l, p]] * G, axis=1) * xr[NF + p:NF + p + 1, :]
                    acc = t if acc is None else acc + t
                h = acc + _dot(vm_ref[l], jnp.concatenate(x[s][nrem:], axis=0))
                xf = xr[:NF + 1]
                row = lax.broadcasted_iota(jnp.int32, xf.shape, 0)
                xf = jnp.where(row == NF, 1.0, xf)
                rhs2[s] = jnp.concatenate([xf, h], axis=0).astype(BF16)
            else:
                r0 = c * half
                y = _dot(l2_ref[l, r0:r0 + half], rhs2[s])
                for r in range(r0, r0 + half, PIECE):
                    j = r // PIECE
                    new = x[s][j].astype(F32) + x0[s][j] * y[r - r0:r - r0 + PIECE]
                    if l == L - 1:
                        obuf[i, rows[j]:rows[j] + PIECE, :] = new.astype(obuf.dtype)
                    else:
                        x[s][j] = new.astype(x[s][j].dtype)
                if l == L - 1 and c == 1:
                    o_copy(i).start()

    for cp in w_copies(0):
        cp.start()
    for i in range(FIRST):
        x_copy(i, 0).start()
    for cp in w_copies(1):
        cp.start(priority=1)
    for cp in w_copies(0):
        cp.wait()
    for i in range(FIRST):
        x_copy(i, 0).wait()
    for i in range(FIRST, FIRST + PER):
        x_copy(i, 1).start(priority=1)
    block(0, FIRST, True)

    nloop = (NS - FIRST) // PER

    def body(it, carry):
        base = FIRST + it * PER
        for j in range(PER):
            x_copy(base + j, (it + 1) % 2).wait()

        @pl.when(it + 1 < nloop)
        def _():
            for j in range(PER):
                x_copy(base + PER + j, it % 2).start()

        block(base, PER, False)
        return carry

    lax.fori_loop(0, nloop, body, 0)
    pltpu.make_async_copy(obuf, obuf, osem.at[0]).wait()


@jax.jit
def pallas_standalone__cross_network_dcn_v2__recsys_kernel(
    x0: jax.Array,
    U: jax.Array,
    V: jax.Array,
    bs: jax.Array,
):
    B, D = x0.shape
    L, _, R = U.shape
    KM = (D // MXU) * MXU
    NP = D - KM - (MXU - R - 1)
    NS = B // SET
    assert NS * SET == B and (NS - FIRST) % PER == 0
    hbm = pl.BlockSpec(memory_space=pl.ANY)
    out_t = pl.pallas_call(
        _kernel,
        in_specs=[hbm] * 4,
        out_specs=hbm,
        out_shape=jax.ShapeDtypeStruct((D, B), x0.dtype),
        scratch_shapes=[
            pltpu.VMEM((NS, D, SET), x0.dtype),
            pltpu.VMEM((NS, D, SET), x0.dtype),
            pltpu.VMEM(U.shape, U.dtype),
            pltpu.VMEM(V.shape, V.dtype),
            pltpu.VMEM(bs.shape, bs.dtype),
            pltpu.VMEM((L, R, KM), F32),
            pltpu.VMEM((L, D, MXU), BF16),
            pltpu.VMEM((L, NP, R, MXU), F32),
            pltpu.SemaphoreType.DMA((2,)),
            pltpu.SemaphoreType.DMA((1,)),
            pltpu.SemaphoreType.DMA((2,)),
        ],
        compiler_params=pltpu.CompilerParams(
            vmem_limit_bytes=100 * 1024 * 1024, disable_bounds_checks=True),
    )(x0.T, U, V, bs)
    return out_t.T
```

```python
import jax
import jax.numpy as jnp
from jax import lax
import jax.experimental.pallas as pl
import jax.experimental.pallas.tpu as pltpu

F32 = jnp.float32
BF16 = jnp.bfloat16

MXU = 128
NMXU = 4
SET = NMXU * MXU
PIECE = 16
FIRST = 2
PER = 6


def _dot(a, b):
    return lax.dot_general(a, b, (((1,), (0,)), ((), ())), preferred_element_type=F32)


def _schedule(nsets, nlayers):
    phases = [[], []]
    for s in range(nsets):
        for l in range(nlayers):
            phases[s % 2] += [("V", s, l), ("U", s, l)]
    order = []
    for t in range(max(len(phases[0]), len(phases[1]) + 1)):
        a = phases[0][t] if t < len(phases[0]) else None
        b = phases[1][t - 1] if 0 <= t - 1 < len(phases[1]) else None
        v = [("V", p[1], p[2], 0) for p in (a, b) if p and p[0] == "V"]
        u = [p for p in (a, b) if p and p[0] == "U"]
        u0 = [("U", p[1], p[2], 0) for p in u]
        u1 = [("U", p[1], p[2], 1) for p in u]
        order += (v + u0 + u1) if t == 1 else (u0 + v + u1)
    return order


def _first_schedule(nlayers):
    head = [("W", 0), ("P", 0), ("V", 0, 0, 0), ("U", 0, 0, 0), ("U", 0, 0, 1),
            ("W", 1), ("V", 1, 0, 0), ("P", 1), ("V", 0, 1, 0), ("U", 1, 0, 0), ("U", 1, 0, 1)]
    order = list(head)
    for op in _schedule(FIRST, nlayers):
        if op in head:
            continue
        if op[0] == "V" and op[1] == 0:
            if op[2] == 2:
                order.append(("W", 2))
            order.append(("P", op[2]))
        order.append(op)
    return order


def _kernel(x_hbm, u_hbm, v_hbm, b_hbm, o_hbm,
            xbuf, obuf, u_ref, v_ref, b_ref, vm_ref, uf_ref, vp_ref, bb_ref,
            xsem, osem, wsem):
    L, D, R = u_hbm.shape
    NS = xbuf.shape[0]
    KM = (D // MXU) * MXU
    NF = MXU - R
    NP = D - KM - NF
    half = D // 2

    def cols(i):
        start = i * SET if isinstance(i, int) else pl.multiple_of(i * SET, SET)
        return pl.ds(start, SET)

    def x_copy(i, sem):
        return pltpu.make_async_copy(x_hbm.at[:, cols(i)], xbuf.at[i], sem)

    def o_copy(i, r0, r1):
        rows = pl.ds(r0, r1 - r0)
        return pltpu.make_async_copy(obuf.at[i, rows], o_hbm.at[rows, cols(i)], osem.at[0])

    def w_copies(l0, l1, sem):
        layers = pl.ds(l0, l1 - l0)
        return [pltpu.make_async_copy(v_hbm.at[layers], v_ref.at[layers], sem),
                pltpu.make_async_copy(u_hbm.at[layers], u_ref.at[layers], sem)]

    def stage(j):
        sem = wsem.at[j]
        if j == 0:
            return w_copies(0, 1, sem) + [pltpu.make_async_copy(b_hbm, b_ref, sem), x_copy(0, sem)]
        if j == 1:
            return [x_copy(1, sem)] + w_copies(1, 2, sem)
        return w_copies(2, L, sem)

    def prepare(l, b_t):
        v = v_ref[l].astype(F32)
        vm_ref[l] = v[:, :KM]
        vrest = jnp.concatenate([v[:, KM:], jnp.zeros((R, MXU - (D - KM)), F32)], axis=1)
        for p in range(NP):
            vp_ref[l, p] = jnp.broadcast_to(vrest[:, NF + p:NF + p + 1], (R, MXU))
        lane = lax.broadcasted_iota(jnp.int32, (R, MXU), 1)
        row = lax.broadcasted_iota(jnp.int32, (R, MXU), 0)
        rhs = jnp.where(lane < NF, vrest, (lane == row + NF).astype(F32)).astype(BF16)
        u = u_ref[l].astype(F32)
        q = D // NMXU
        uf = jnp.concatenate([_dot(u[j * q:(j + 1) * q], rhs) for j in range(NMXU)], axis=0)
        uf_ref[l] = uf.astype(BF16)
        bb_ref[l] = jnp.broadcast_to(b_t[:, l:l + 1], (D, MXU))

    def block(base, order):
        x0, x, rhs = {}, {}, {}
        b_t = None
        for op in order:
            if op[0] == "W":
                for copy in stage(op[1]):
                    copy.wait()
                if op[1] == 0:
                    for copy in stage(2):
                        copy.start(priority=1)
                    b_t = jnp.transpose(b_ref[...].astype(F32))
                else:
                    first = FIRST + (op[1] - 1) * PER
                    for i in range(first, first + PER):
                        x_copy(i, xsem.at[op[1] - 1]).start(priority=1)
            elif op[0] == "P":
                prepare(op[1], b_t)
            elif op[0] == "V":
                _, s, l, _ = op
                if l == 0:
                    raw = {r: xbuf[base + s, r:r + PIECE, :] for r in range(0, D, PIECE)}
                    x0[s] = {r: a.astype(F32) for r, a in raw.items()}
                    x[s] = {r: (raw[r] if r < KM else x0[s][r]) for r in raw}
                rest = jnp.concatenate([x[s][r] for r in range(KM, D, PIECE)], axis=0)
                h = None
                for p in range(NP):
                    t = jnp.concatenate([vp_ref[l, p]] * NMXU, axis=1) * rest[NF + p:NF + p + 1, :]
                    h = t if h is None else h + t
                main = jnp.concatenate([x[s][r] for r in range(0, KM, PIECE)], axis=0)
                h = h + _dot(vm_ref[l], main)
                rhs[s] = jnp.concatenate([rest[:NF], h], axis=0).astype(BF16)
            else:
                _, s, l, c = op
                r0, r1 = c * half, (c + 1) * half
                mid = r0 + (half // PIECE + 1) // 2 * PIECE
                y = _dot(uf_ref[l, r0:r1], rhs[s])
                for r in range(r0, r1, PIECE):
                    bias = jnp.concatenate([bb_ref[l, r:r + PIECE]] * NMXU, axis=1)
                    new = x[s][r].astype(F32) + x0[s][r] * (y[r - r0:r - r0 + PIECE] + bias)
                    if l < L - 1:
                        x[s][r] = new.astype(x[s][r].dtype)
                        continue
                    obuf[base + s, r:r + PIECE, :] = new.astype(obuf.dtype)
                    if r + PIECE == mid:
                        o_copy(base + s, r0, mid).start()
                    if r + PIECE == r1:
                        o_copy(base + s, mid, r1).start()

    for copy in stage(0):
        copy.start()
    for copy in stage(1):
        copy.start(priority=1)
    block(0, _first_schedule(L))

    nloop = (NS - FIRST) // PER

    def body(it, carry):
        base = FIRST + it * PER
        sem = xsem.at[it & 1]
        batch = xbuf.at[pl.ds(base, PER)]
        pltpu.make_async_copy(batch, batch, sem).wait()
        block(base, _schedule(PER, L))

        @pl.when(it + 2 < nloop)
        def _():
            for j in range(PER):
                x_copy(base + 2 * PER + j, sem).start()

        return carry

    lax.fori_loop(0, nloop, body, 0)
    pltpu.make_async_copy(obuf, obuf, osem.at[0]).wait()


@jax.jit
def pallas_standalone__cross_network_dcn_v2__recsys_kernel(
    x0: jax.Array,
    U: jax.Array,
    V: jax.Array,
    bs: jax.Array,
):
    B, D = x0.shape
    L, _, R = U.shape
    KM = (D // MXU) * MXU
    NP = D - KM - (MXU - R)
    NS = B // SET
    assert NS * SET == B and (NS - FIRST) % PER == 0 and NS >= FIRST + 2 * PER and L >= 3
    hbm = pl.BlockSpec(memory_space=pl.ANY)
    out_t = pl.pallas_call(
        _kernel,
        in_specs=[hbm] * 4,
        out_specs=hbm,
        out_shape=jax.ShapeDtypeStruct((D, B), x0.dtype),
        scratch_shapes=[
            pltpu.VMEM((NS, D, SET), x0.dtype),
            pltpu.VMEM((NS, D, SET), x0.dtype),
            pltpu.VMEM(U.shape, U.dtype),
            pltpu.VMEM(V.shape, V.dtype),
            pltpu.VMEM(bs.shape, bs.dtype),
            pltpu.VMEM((L, R, KM), F32),
            pltpu.VMEM((L, D, MXU), BF16),
            pltpu.VMEM((L, NP, R, MXU), F32),
            pltpu.VMEM((L, D, MXU), F32),
            pltpu.SemaphoreType.DMA((2,)),
            pltpu.SemaphoreType.DMA((1,)),
            pltpu.SemaphoreType.DMA((3,)),
        ],
        compiler_params=pltpu.CompilerParams(
            vmem_limit_bytes=100 * 1024 * 1024,
            disable_bounds_checks=True,
            disable_semaphore_checks=True,
        ),
    )(x0.T, U, V, bs)
    return out_t.T
```

```python
import jax
import jax.numpy as jnp
from jax import lax
import jax.experimental.pallas as pl
import jax.experimental.pallas.tpu as pltpu

F32 = jnp.float32
BF16 = jnp.bfloat16

MXU = 128
NMXU = 4
SET = NMXU * MXU
PIECE = 16
FIRST = 2
PER = 6


def _dot(a, b):
    return lax.dot_general(a, b, (((1,), (0,)), ((), ())), preferred_element_type=F32)


def _schedule(nsets, nlayers):
    phases = [[], []]
    for s in range(nsets):
        for l in range(nlayers):
            phases[s % 2] += [("V", s, l), ("U", s, l)]
    order = []
    for t in range(max(len(phases[0]), len(phases[1]) + 1)):
        a = phases[0][t] if t < len(phases[0]) else None
        b = phases[1][t - 1] if 0 <= t - 1 < len(phases[1]) else None
        v = [("V", p[1], p[2], 0) for p in (a, b) if p and p[0] == "V"]
        u = [p for p in (a, b) if p and p[0] == "U"]
        u0 = [("U", p[1], p[2], 0) for p in u]
        u1 = [("U", p[1], p[2], 1) for p in u]
        order += (v + u0 + u1) if t == 1 else (u0 + v + u1)
    return order


def _first_schedule(nlayers):
    order = [("W", 0), ("PV", 0), ("V", 0, 0, 0), ("PU", 0), ("U", 0, 0, 0), ("U", 0, 0, 1),
             ("W", 1), ("V", 1, 0, 0), ("PV", 1), ("V", 0, 1, 0), ("PU", 1),
             ("U", 1, 0, 0), ("U", 1, 0, 1)]
    for op in [op for op in _schedule(FIRST, nlayers) if op not in order]:
        if op == ("U", 0, 1, 1):
            order.append(("W", 2))
        if op == ("V", 0, 2, 0):
            order += [("PV", 2), ("PU", 2)]
        order.append(op)
        if op[:2] == ("V", 0) and 2 <= op[2] < nlayers - 1:
            order += [("PV", op[2] + 1), ("PU", op[2] + 1)]
    return order


def _kernel(x_hbm, u_hbm, v_hbm, b_hbm, o_hbm,
            xbuf, obuf, u_ref, v_ref, b_ref, vm_ref, uf_ref, vp_ref, bb_ref,
            xsem, osem, wsem):
    L, D, R = u_hbm.shape
    NS = xbuf.shape[0]
    KM = (D // MXU) * MXU
    NF = MXU - R
    NP = D - KM - NF
    half = D // 2

    def cols(i):
        start = i * SET if isinstance(i, int) else pl.multiple_of(i * SET, SET)
        return pl.ds(start, SET)

    def x_copy(i, sem):
        return pltpu.make_async_copy(x_hbm.at[:, cols(i)], xbuf.at[i], sem)

    def o_copy(i, r0, r1):
        rows = pl.ds(r0, r1 - r0)
        return pltpu.make_async_copy(obuf.at[i, rows], o_hbm.at[rows, cols(i)], osem.at[0])

    def w_copies(l0, l1, sem):
        layers = pl.ds(l0, l1 - l0)
        return [pltpu.make_async_copy(v_hbm.at[layers], v_ref.at[layers], sem),
                pltpu.make_async_copy(u_hbm.at[layers], u_ref.at[layers], sem)]

    def stage(j):
        sem = wsem.at[j]
        if j == 0:
            return w_copies(0, 1, sem) + [pltpu.make_async_copy(b_hbm, b_ref, sem), x_copy(0, sem)]
        if j == 1:
            return [x_copy(1, sem)] + w_copies(1, 2, sem)
        return w_copies(2, L, sem)

    def prepare_v(l):
        v = v_ref[l].astype(F32)
        vm_ref[l] = v[:, :KM]
        vrest = jnp.concatenate([v[:, KM:], jnp.zeros((R, MXU - (D - KM)), F32)], axis=1)
        for p in range(NP):
            vp_ref[l, p] = jnp.broadcast_to(vrest[:, NF + p:NF + p + 1], (R, MXU))
        return v[:, KM:KM + NF]

    def prepare_u(l, vf, b_t):
        uvf_t = lax.dot_general(jnp.transpose(vf), u_ref[l], (((1,), (1,)), ((), ())),
                                preferred_element_type=F32)
        uvf = jnp.transpose(jnp.concatenate([jnp.zeros((R, D), F32), uvf_t], axis=0))
        u = jnp.concatenate([u_ref[l].astype(F32), jnp.zeros((D, NF), F32)], axis=1)
        uf_ref[l] = (u + uvf).astype(BF16)
        bb_ref[l] = jnp.broadcast_to(b_t[:, l:l + 1], (D, MXU))

    def block(base, order):
        x0, x, rhs, vf = {}, {}, {}, {}
        b_t = None
        for op in order:
            if op[0] == "W":
                for copy in stage(op[1]):
                    copy.wait()
                if op[1] == 0:
                    for copy in stage(2):
                        copy.start(priority=1)
                    b_t = jnp.transpose(b_ref[...].astype(F32))
                else:
                    first = FIRST + (op[1] - 1) * PER
                    for i in range(first, first + PER):
                        x_copy(i, xsem.at[op[1] - 1]).start(priority=1)
            elif op[0] == "PV":
                vf[op[1]] = prepare_v(op[1])
            elif op[0] == "PU":
                prepare_u(op[1], vf[op[1]], b_t)
            elif op[0] == "V":
                _, s, l, _ = op
                if l == 0:
                    raw = {r: xbuf[base + s, r:r + PIECE, :] for r in range(0, D, PIECE)}
                    x0[s] = {r: a.astype(F32) for r, a in raw.items()}
                    x[s] = {r: (raw[r] if r < KM else x0[s][r]) for r in raw}
                rest = jnp.concatenate([x[s][r] for r in range(KM, D, PIECE)], axis=0)
                h = None
                for p in range(NP):
                    t = jnp.concatenate([vp_ref[l, p]] * NMXU, axis=1) * rest[NF + p:NF + p + 1, :]
                    h = t if h is None else h + t
                main = jnp.concatenate([x[s][r] for r in range(0, KM, PIECE)], axis=0)
                h = h + _dot(vm_ref[l], main)
                rhs[s] = jnp.concatenate([h, rest[:NF]], axis=0).astype(BF16)
            else:
                _, s, l, c = op
                r0, r1 = c * half, (c + 1) * half
                mid = r0 + (half // PIECE + 1) // 2 * PIECE
                y = _dot(uf_ref[l, r0:r1], rhs[s])
                for r in range(r0, r1, PIECE):
                    bias = jnp.concatenate([bb_ref[l, r:r + PIECE]] * NMXU, axis=1)
                    new = x[s][r].astype(F32) + x0[s][r] * (y[r - r0:r - r0 + PIECE] + bias)
                    if l < L - 1:
                        x[s][r] = new.astype(x[s][r].dtype)
                        continue
                    obuf[base + s, r:r + PIECE, :] = new.astype(obuf.dtype)
                    if r + PIECE == mid:
                        o_copy(base + s, r0, mid).start()
                    if r + PIECE == r1:
                        o_copy(base + s, mid, r1).start()

    for copy in stage(0):
        copy.start()
    for copy in stage(1):
        copy.start(priority=1)
    block(0, _first_schedule(L))

    nloop = (NS - FIRST) // PER

    def body(it, carry):
        base = FIRST + it * PER
        sem = xsem.at[it & 1]
        batch = xbuf.at[pl.ds(base, PER)]
        pltpu.make_async_copy(batch, batch, sem).wait()
        block(base, _schedule(PER, L))

        @pl.when(it + 2 < nloop)
        def _():
            for j in range(PER):
                x_copy(base + 2 * PER + j, sem).start()

        return carry

    lax.fori_loop(0, nloop, body, 0)
    pltpu.make_async_copy(obuf, obuf, osem.at[0]).wait()


@jax.jit
def pallas_standalone__cross_network_dcn_v2__recsys_kernel(
    x0: jax.Array,
    U: jax.Array,
    V: jax.Array,
    bs: jax.Array,
):
    B, D = x0.shape
    L, _, R = U.shape
    KM = (D // MXU) * MXU
    NP = D - KM - (MXU - R)
    NS = B // SET
    assert NS * SET == B and (NS - FIRST) % PER == 0 and NS >= FIRST + 2 * PER and L >= 3
    hbm = pl.BlockSpec(memory_space=pl.ANY)
    out_t = pl.pallas_call(
        _kernel,
        in_specs=[hbm] * 4,
        out_specs=hbm,
        out_shape=jax.ShapeDtypeStruct((D, B), x0.dtype),
        scratch_shapes=[
            pltpu.VMEM((NS, D, SET), x0.dtype),
            pltpu.VMEM((NS, D, SET), x0.dtype),
            pltpu.VMEM(U.shape, U.dtype),
            pltpu.VMEM(V.shape, V.dtype),
            pltpu.VMEM(bs.shape, bs.dtype),
            pltpu.VMEM((L, R, KM), F32),
            pltpu.VMEM((L, D, MXU), BF16),
            pltpu.VMEM((L, NP, R, MXU), F32),
            pltpu.VMEM((L, D, MXU), F32),
            pltpu.SemaphoreType.DMA((2,)),
            pltpu.SemaphoreType.DMA((1,)),
            pltpu.SemaphoreType.DMA((3,)),
        ],
        compiler_params=pltpu.CompilerParams(
            vmem_limit_bytes=100 * 1024 * 1024,
            disable_bounds_checks=True,
        ),
    )(x0.T, U, V, bs)
    return out_t.T
```
